```python
import os as _os
_os.environ.setdefault("JAX_PLATFORMS", "cpu")
import jax
import jax.numpy as jnp

def _softmax(x, axis=-1):
    return jax.nn.softmax(x, axis=axis)
def _gelu(x):
    return jax.nn.gelu(x, approximate=True)
def _silu(x):
    return jax.nn.silu(x)
def _sigmoid(x):
    return jax.nn.sigmoid(x)
def _layernorm(x, axis=-1, eps=1e-5):
    m = jnp.mean(x, axis=axis, keepdims=True)
    v = jnp.var(x, axis=axis, keepdims=True)
    return (x - m) / jnp.sqrt(v + eps)
def _scatter_add(tgt, idx, src, axis=0):
    return tgt.at[idx].add(src)
def _segment_sum(src, seg, n):
    return jax.ops.segment_sum(src, seg, n)
class _Rng:
    def __init__(self, key):
        self._k = key
    def _next(self):
        self._k, sub = jax.random.split(self._k)
        return sub
    def normal(self, shape):
        return jax.random.normal(self._next(), shape, dtype=jnp.bfloat16)
    def randint(self, lo, hi, shape):
        return jax.random.randint(self._next(), shape, lo, hi, dtype=jnp.int32)
    def uniform(self, shape, lo=0.0, hi=1.0):
        return jax.random.uniform(self._next(), shape, jnp.bfloat16, lo, hi)
    def permutation(self, n):
        return jax.random.permutation(self._next(), n)


kernel_name = 'concat_heads__mha_block_cached__mha_block_cached__near_ridge'

def setup_inputs():
    _rng = _Rng(jax.random.key(int.from_bytes(__import__("os").urandom(4), "little")))
    _w = (lambda a: (lambda t: t.astype(jnp.bfloat16) if jnp.issubdtype(t.dtype, jnp.floating) else t)(jnp.asarray(a)))
    def _A_setup():
        B, Sq, D = 8, 144, 640
        H, Sk, Dh = 32, 512, 128
        return {
            "x": _w((lambda *s: _rng.normal(s) * 0.8)(B, Sq, D)),
            "k_cache": _w((lambda *s: _rng.normal(s) * 0.8)(B, H, Sk, Dh)),
            "v_cache": _w((lambda *s: _rng.normal(s) * 0.05)(B, H, Sk, Dh)),
            "wq": _w((lambda *s: _rng.normal(s) * 0.8)(D, H * Dh) * (D ** -0.5)),
            "wo": _w((lambda *s: _rng.normal(s) * 0.05)(H * Dh, D) * ((H * Dh) ** -0.5)),
        }
    _A_in = _A_setup()

    def _B_setup():
        B, Sq, D = 8, 144, 640
        H, Sk, Dh = 32, 512, 128
        return {
            "x": _w((lambda *s: _rng.normal(s) * 0.8)(B, Sq, D)),
            "k_cache": _w((lambda *s: _rng.normal(s) * 0.8)(B, H, Sk, Dh)),
            "v_cache": _w((lambda *s: _rng.normal(s) * 0.05)(B, H, Sk, Dh)),
            "wq": _w((lambda *s: _rng.normal(s) * 0.8)(D, H * Dh) * (D ** -0.5)),
            "wo": _w((lambda *s: _rng.normal(s) * 0.05)(H * Dh, D) * ((H * Dh) ** -0.5)),
        }
    _B_in = _B_setup()

    return {
        "A_x": _A_in["x"],
        "A_k_cache": _A_in["k_cache"],
        "A_v_cache": _A_in["v_cache"],
        "A_wq": _A_in["wq"],
        "A_wo": _A_in["wo"],
        "B_x": _B_in["x"],
        "B_k_cache": _B_in["k_cache"],
        "B_v_cache": _B_in["v_cache"],
        "B_wq": _B_in["wq"],
        "B_wo": _B_in["wo"],
    }

def reference(A_x, A_k_cache, A_v_cache, A_wq, A_wo, B_x, B_k_cache, B_v_cache, B_wq, B_wo):
    def _A_ref(x, k_cache, v_cache, wq, wo):
        B, Sq, D = x.shape
        H, Dh = 32, 128
        q = (lambda x, *d: x.transpose(*d))((x @ wq).reshape(B, Sq, H, Dh), 0, 2, 1, 3)
        scores = jnp.einsum("bhqd,bhkd->bhqk", q, k_cache) * (Dh ** -0.5)
        p = _softmax(scores, axis=-1)
        o = jnp.einsum("bhqk,bhkd->bhqd", p, v_cache)
        return (lambda x, *d: x.transpose(*d))(o, 0, 2, 1, 3).reshape(B, Sq, H * Dh) @ wo

    def _B_ref(x, k_cache, v_cache, wq, wo):
        B, Sq, D = x.shape
        H, Dh = 32, 128
        q = (lambda x, *d: x.transpose(*d))((x @ wq).reshape(B, Sq, H, Dh), 0, 2, 1, 3)
        scores = jnp.einsum("bhqd,bhkd->bhqk", q, k_cache) * (Dh ** -0.5)
        p = _softmax(scores, axis=-1)
        o = jnp.einsum("bhqk,bhkd->bhqd", p, v_cache)
        return (lambda x, *d: x.transpose(*d))(o, 0, 2, 1, 3).reshape(B, Sq, H * Dh) @ wo

    a = _A_ref(A_x, A_k_cache, A_v_cache, A_wq, A_wo)
    b = _B_ref(B_x, B_k_cache, B_v_cache, B_wq, B_wo)
    return jnp.concatenate([a, b], axis=-1)
```

```python
import functools

import jax
import jax.numpy as jnp
import jax.experimental.pallas as pl
import jax.experimental.pallas.tpu as pltpu

_G = 8


def _mha_step(x_ref, k_ref, v_ref, wq_ref, wo_ref, o_ref, acc_ref, *, hg, n_hg, G, Dh):
    x = x_ref[0]
    scale = Dh ** -0.5

    @pl.when(hg == 0)
    def _():
        acc_ref[...] = jnp.zeros_like(acc_ref)

    os = []
    for g in range(G):
        col = pl.multiple_of((hg * G + g) * Dh, Dh)
        wq_h = wq_ref[:, pl.ds(col, Dh)]
        q = jnp.dot(x, wq_h, preferred_element_type=jnp.float32)
        q = (q * scale).astype(jnp.bfloat16)
        k = k_ref[0, g]
        s = jax.lax.dot_general(q, k, (((1,), (1,)), ((), ())),
                                preferred_element_type=jnp.float32)
        m = jnp.max(s, axis=-1, keepdims=True)
        p = jnp.exp(s - m)
        l = jnp.sum(p, axis=-1, keepdims=True)
        o = jnp.dot(p.astype(jnp.bfloat16), v_ref[0, g],
                    preferred_element_type=jnp.float32)
        o = o / l
        os.append(o.astype(jnp.bfloat16))
    o_all = jnp.concatenate(os, axis=-1)
    row = pl.multiple_of(hg * G * Dh, G * Dh)
    wo_g = wo_ref[pl.ds(row, G * Dh), :]
    acc_ref[...] += jnp.dot(o_all, wo_g, preferred_element_type=jnp.float32)

    @pl.when(hg == n_hg - 1)
    def _():
        o_ref[0] = acc_ref[...].astype(o_ref.dtype)


def _kernel(ax_ref, ak_ref, av_ref, awq_ref, awo_ref,
            bx_ref, bk_ref, bv_ref, bwq_ref, bwo_ref,
            o_ref, acc_ref, *, G, Dh, n_hg):
    blk = pl.program_id(0)
    hg = pl.program_id(2)

    @pl.when(blk == 0)
    def _():
        _mha_step(ax_ref, ak_ref, av_ref, awq_ref, awo_ref, o_ref, acc_ref,
                  hg=hg, n_hg=n_hg, G=G, Dh=Dh)

    @pl.when(blk == 1)
    def _():
        _mha_step(bx_ref, bk_ref, bv_ref, bwq_ref, bwo_ref, o_ref, acc_ref,
                  hg=hg, n_hg=n_hg, G=G, Dh=Dh)


@jax.jit
def pallas_concat_heads__mha_block_cached__mha_block_cached__near_ridge_kernel(
    A_x: jax.Array,
    A_k_cache: jax.Array,
    A_v_cache: jax.Array,
    A_wq: jax.Array,
    A_wo: jax.Array,
    B_x: jax.Array,
    B_k_cache: jax.Array,
    B_v_cache: jax.Array,
    B_wq: jax.Array,
    B_wo: jax.Array,
):
    B, Sq, D = A_x.shape
    _, H, Sk, Dh = A_k_cache.shape
    G = _G
    n_hg = H // G

    def x_map_a(blk, b, hg):
        return (jnp.where(blk == 0, b, B - 1), 0, 0)

    def x_map_b(blk, b, hg):
        return (jnp.where(blk == 1, b, 0), 0, 0)

    def kv_map_a(blk, b, hg):
        return (jnp.where(blk == 0, b, B - 1), jnp.where(blk == 0, hg, n_hg - 1), 0, 0)

    def kv_map_b(blk, b, hg):
        return (jnp.where(blk == 1, b, 0), jnp.where(blk == 1, hg, 0), 0, 0)

    x_spec_a = pl.BlockSpec((1, Sq, D), x_map_a)
    x_spec_b = pl.BlockSpec((1, Sq, D), x_map_b)
    kv_spec_a = pl.BlockSpec((1, G, Sk, Dh), kv_map_a)
    kv_spec_b = pl.BlockSpec((1, G, Sk, Dh), kv_map_b)
    wq_spec = pl.BlockSpec((D, H * Dh), lambda blk, b, hg: (0, 0),
                           pipeline_mode=pl.Buffered(1))
    wo_spec = pl.BlockSpec((H * Dh, D), lambda blk, b, hg: (0, 0),
                           pipeline_mode=pl.Buffered(1))
    out_spec = pl.BlockSpec((1, Sq, D), lambda blk, b, hg: (b, 0, blk))

    kernel = functools.partial(_kernel, G=G, Dh=Dh, n_hg=n_hg)
    return pl.pallas_call(
        kernel,
        grid=(2, B, n_hg),
        in_specs=[x_spec_a, kv_spec_a, kv_spec_a, wq_spec, wo_spec,
                  x_spec_b, kv_spec_b, kv_spec_b, wq_spec, wo_spec],
        out_specs=out_spec,
        out_shape=jax.ShapeDtypeStruct((B, Sq, 2 * D), A_x.dtype),
        scratch_shapes=[pltpu.VMEM((Sq, D), jnp.float32)],
        compiler_params=pltpu.CompilerParams(
            dimension_semantics=("arbitrary", "arbitrary", "arbitrary"),
            vmem_limit_bytes=100 * 1024 * 1024,
        ),
    )(A_x, A_k_cache, A_v_cache, A_wq, A_wo,
      B_x, B_k_cache, B_v_cache, B_wq, B_wo)
```

```python
import functools
import os

import jax
import jax.numpy as jnp
from jax import lax
import jax.experimental.pallas as pl
import jax.experimental.pallas.tpu as pltpu

_G = 8
_NS = 4
LOG2E = 1.4426950408889634


def _log2(n):
    l = n.bit_length() - 1
    assert (1 << l) == n, n
    return l


def _kernel(xa, ka, va, wqa, woa, xb, kb, vb, wqb, wob, out_hbm,
            xbuf, kbuf, vbuf, wqbuf, wobuf, acc, obuf,
            x_sems, kv_sems, w_sems, o_sems, *, B, Sq, D, H, Sk, Dh, G, NS):
    n_hg = H // G
    NU = 2 * n_hg * B
    NW = 2 * n_hg
    GD = G * Dh
    lb, lh = _log2(B), _log2(n_hg)
    assert n_hg > 1 and NS == 4 and B >= 8

    def dec(u):
        return u >> (lb + lh), (u >> lb) & (n_hg - 1), u & (B - 1)

    def x_copy(x_hbm, blk_static, b):
        return pltpu.make_async_copy(x_hbm.at[b], xbuf.at[blk_static, b],
                                     x_sems.at[blk_static * B + b])

    def start_kv(k_hbm, v_hbm, b, hg, slot):
        h0 = pl.multiple_of(hg * G, G)
        pltpu.make_async_copy(k_hbm.at[b, pl.ds(h0, G)], kbuf.at[slot],
                              kv_sems.at[2 * slot]).start()
        pltpu.make_async_copy(v_hbm.at[b, pl.ds(h0, G)], vbuf.at[slot],
                              kv_sems.at[2 * slot + 1]).start()

    def issue_kv(u):
        blk, hg, b = dec(u)
        slot = u & (NS - 1)

        @pl.when(blk == 0)
        def _():
            start_kv(ka, va, b, hg, slot)

        @pl.when(blk == 1)
        def _():
            start_kv(kb, vb, b, hg, slot)

    def static_unit(u0):
        blk, hg, b = dec(u0)
        assert blk == 0
        if hg == 0:
            x_copy(xa, 0, b).start()
        start_kv(ka, va, b, hg, u0 & (NS - 1))

    def wq_copy(wq_hbm, hg, wslot):
        c0 = pl.multiple_of(hg * GD, GD)
        return pltpu.make_async_copy(wq_hbm.at[:, pl.ds(c0, GD)], wqbuf.at[wslot],
                                     w_sems.at[2 * wslot])

    def wo_copy(wo_hbm, hg, wslot):
        c0 = pl.multiple_of(hg * GD, GD)
        return pltpu.make_async_copy(wo_hbm.at[pl.ds(c0, GD), :], wobuf.at[wslot],
                                     w_sems.at[2 * wslot + 1])

    def issue_w(w):
        blk = w >> lh
        hg = w & (n_hg - 1)
        wslot = w & 1

        @pl.when(blk == 0)
        def _():
            wq_copy(wqa, hg, wslot).start(priority=1)
            wo_copy(woa, hg, wslot).start(priority=1)

        @pl.when(blk == 1)
        def _():
            wq_copy(wqb, hg, wslot).start(priority=1)
            wo_copy(wob, hg, wslot).start(priority=1)

    def out_copy(blk_static, b):
        return pltpu.make_async_copy(
            obuf.at[blk_static, b],
            out_hbm.at[b, :, pl.ds(blk_static * D, D)],
            o_sems.at[blk_static * B + b])

    qscale = (Dh ** -0.5) * LOG2E

    def waits(u):
        blk, hg, b = dec(u)
        w = u >> lb
        slot = u & (NS - 1)
        wslot = w & 1

        @pl.when(hg == 0)
        def _():
            pltpu.make_async_copy(xbuf.at[blk, b], xbuf.at[blk, b],
                                  x_sems.at[blk * B + b]).wait()

        @pl.when(b == 0)
        def _():
            pltpu.make_async_copy(wqbuf.at[wslot], wqbuf.at[wslot], w_sems.at[2 * wslot]).wait()
            pltpu.make_async_copy(wobuf.at[wslot], wobuf.at[wslot], w_sems.at[2 * wslot + 1]).wait()

        pltpu.make_async_copy(kbuf.at[slot], kbuf.at[slot], kv_sems.at[2 * slot]).wait()
        pltpu.make_async_copy(vbuf.at[slot], vbuf.at[slot], kv_sems.at[2 * slot + 1]).wait()

    def compute(u):
        blk, hg, b = dec(u)
        w = u >> lb
        slot = u & (NS - 1)
        wslot = w & 1

        x = xbuf[blk, b]
        q_all = jnp.dot(x, wqbuf[wslot], preferred_element_type=jnp.float32)
        q_all = (q_all * qscale).astype(jnp.bfloat16)

        def qk(g):
            return lax.dot_general(q_all[:, g * Dh:(g + 1) * Dh], kbuf[slot, g],
                                   (((1,), (1,)), ((), ())),
                                   preferred_element_type=jnp.float32)

        def sm_pv(g, s):
            m = jnp.max(s, axis=-1, keepdims=True)
            p = jnp.exp2(s - m)
            l = jnp.sum(p, axis=-1, keepdims=True)
            o = jnp.dot(p.astype(jnp.bfloat16), vbuf[slot, g],
                        preferred_element_type=jnp.float32)
            r = pl.reciprocal(l, approx=True)
            r = r * (2.0 - l * r)
            return (o * r).astype(jnp.bfloat16)

        os_ = []
        s_cur = qk(0)
        for g in range(G):
            s_next = qk(g + 1) if g + 1 < G else None
            os_.append(sm_pv(g, s_cur))
            s_cur = s_next
        o_all = jnp.concatenate(os_, axis=-1)

        prev = jnp.where(hg == 0, 0.0, acc[b])
        new = prev + jnp.dot(o_all, wobuf[wslot], preferred_element_type=jnp.float32)
        acc[b] = new
        obuf[blk, b] = new.astype(obuf.dtype)

    def starts(u, kv=True):
        blk, hg, b = dec(u)
        w = u >> lb

        if kv:
            @pl.when(u + NS < NU)
            def _():
                issue_kv(u + NS)

        @pl.when(jnp.logical_and(b == B - 1, w + 2 < NW))
        def _():
            issue_w(w + 2)

        @pl.when(jnp.logical_and(hg == n_hg - 1, blk == 0))
        def _():
            out_copy(0, b).start()

        @pl.when(jnp.logical_and(hg == n_hg - 1, blk == 1))
        def _():
            out_copy(1, b).start()

    x_copy(xa, 0, 0).start()
    wq_copy(wqa, 0, 0).start()
    start_kv(ka, va, 0, 0, 0)
    wo_copy(woa, 0, 0).start()

    u = jnp.int32(0)
    waits(u)
    static_unit(1)
    wq_copy(wqa, 1, 1).start(priority=1)
    wo_copy(woa, 1, 1).start(priority=1)
    compute(u)
    starts(u, kv=False)
    static_unit(2)
    static_unit(3)

    u = jnp.int32(1)
    waits(u)
    compute(u)
    starts(u, kv=False)

    us = [jnp.int32(2), jnp.int32(3)]
    for u in us:
        waits(u)
    static_unit(4)
    static_unit(5)
    for u in us:
        compute(u)
    for u in us:
        starts(u)
    x_copy(xa, 0, 6).start()
    x_copy(xa, 0, 7).start()
    for b0 in range(B):
        x_copy(xb, 1, b0).start(priority=1)

    def loop_body(i, carry):
        us = [4 + 2 * i, 5 + 2 * i]
        for u in us:
            waits(u)
        for u in us:
            compute(u)
        for u in us:
            starts(u)
        return carry

    lax.fori_loop(0, (NU - 4) // 2, loop_body, 0)

    for blk_s in range(2):
        for b_s in range(B):
            out_copy(blk_s, b_s).wait()


@jax.jit
def pallas_concat_heads__mha_block_cached__mha_block_cached__near_ridge_kernel(
    A_x, A_k_cache, A_v_cache, A_wq, A_wo, B_x, B_k_cache, B_v_cache, B_wq, B_wo):
    B, Sq, D = A_x.shape
    _, H, Sk, Dh = A_k_cache.shape
    G, NS = _G, _NS
    kernel = functools.partial(_kernel, B=B, Sq=Sq, D=D, H=H, Sk=Sk, Dh=Dh, G=G, NS=NS)
    any_spec = pl.BlockSpec(memory_space=pl.ANY)
    return pl.pallas_call(
        kernel,
        in_specs=[any_spec] * 10,
        out_specs=any_spec,
        out_shape=jax.ShapeDtypeStruct((B, Sq, 2 * D), A_x.dtype),
        scratch_shapes=[
            pltpu.VMEM((2, B, Sq, D), jnp.bfloat16),
            pltpu.VMEM((NS, G, Sk, Dh), jnp.bfloat16),
            pltpu.VMEM((NS, G, Sk, Dh), jnp.bfloat16),
            pltpu.VMEM((2, D, G * Dh), jnp.bfloat16),
            pltpu.VMEM((2, G * Dh, D), jnp.bfloat16),
            pltpu.VMEM((B, Sq, D), jnp.float32),
            pltpu.VMEM((2, B, Sq, D), jnp.bfloat16),
            pltpu.SemaphoreType.DMA((2 * B,)),
            pltpu.SemaphoreType.DMA((2 * NS,)),
            pltpu.SemaphoreType.DMA((4,)),
            pltpu.SemaphoreType.DMA((2 * B,)),
        ],
        compiler_params=pltpu.CompilerParams(
            vmem_limit_bytes=100 * 1024 * 1024,
        ),
    )(A_x, A_k_cache, A_v_cache, A_wq, A_wo,
      B_x, B_k_cache, B_v_cache, B_wq, B_wo)
```

```python
import functools

import jax
import jax.numpy as jnp
from jax import lax
import jax.experimental.pallas as pl
import jax.experimental.pallas.tpu as pltpu

_G = 8
_NS = 4
_LOG2E = 1.4426950408889634


def _log2(n):
    l = n.bit_length() - 1
    assert (1 << l) == n, n
    return l


def _kernel(xa, ka, va, wqa, woa, xb, kb, vb, wqb, wob, out_hbm,
            xbuf, kbuf, vbuf, wqbuf, wobuf, acc, obuf,
            x_sems, kv_sems, w_sems, o_sems, *, B, Sq, D, H, Sk, Dh, G, NS):
    n_hg = H // G
    NU = 2 * n_hg * B
    NW = 2 * n_hg
    GD = G * Dh
    lb, lh = _log2(B), _log2(n_hg)
    assert n_hg > 1 and NS == 4 and B == 8

    def dec(u):
        return u >> (lb + lh), (u >> lb) & (n_hg - 1), u & (B - 1)

    def x_copy(x_hbm, blk_static, b):
        return pltpu.make_async_copy(x_hbm.at[b], xbuf.at[blk_static, b],
                                     x_sems.at[blk_static * B + b])

    def start_kv(k_hbm, v_hbm, b, hg, slot):
        h0 = pl.multiple_of(hg * G, G)
        pltpu.make_async_copy(k_hbm.at[b, pl.ds(h0, G)], kbuf.at[slot],
                              kv_sems.at[2 * slot]).start()
        pltpu.make_async_copy(v_hbm.at[b, pl.ds(h0, G)], vbuf.at[slot],
                              kv_sems.at[2 * slot + 1]).start()

    def issue_kv(u):
        blk, hg, b = dec(u)
        slot = u & (NS - 1)

        @pl.when(blk == 0)
        def _():
            start_kv(ka, va, b, hg, slot)

        @pl.when(blk == 1)
        def _():
            start_kv(kb, vb, b, hg, slot)

    def static_unit(u0):
        blk, hg, b = dec(u0)
        assert blk == 0 and hg == 0
        x_copy(xa, 0, b).start()
        start_kv(ka, va, b, hg, u0 & (NS - 1))

    def wq_copy(wq_hbm, hg, wslot):
        c0 = pl.multiple_of(hg * GD, GD)
        return pltpu.make_async_copy(wq_hbm.at[:, pl.ds(c0, GD)], wqbuf.at[wslot],
                                     w_sems.at[2 * wslot])

    def wo_copy(wo_hbm, hg, wslot):
        c0 = pl.multiple_of(hg * GD, GD)
        return pltpu.make_async_copy(wo_hbm.at[pl.ds(c0, GD), :], wobuf.at[wslot],
                                     w_sems.at[2 * wslot + 1])

    def issue_w(w):
        blk = w >> lh
        hg = w & (n_hg - 1)
        wslot = w & 1

        @pl.when(blk == 0)
        def _():
            wq_copy(wqa, hg, wslot).start(priority=1)
            wo_copy(woa, hg, wslot).start(priority=1)

        @pl.when(blk == 1)
        def _():
            wq_copy(wqb, hg, wslot).start(priority=1)
            wo_copy(wob, hg, wslot).start(priority=1)

    def out_copy(blk_static, b):
        return pltpu.make_async_copy(
            obuf.at[blk_static, b],
            out_hbm.at[b, :, pl.ds(blk_static * D, D)],
            o_sems.at[blk_static * B + b])

    qscale = (Dh ** -0.5) * _LOG2E

    def waits(u):
        blk, hg, b = dec(u)
        w = u >> lb
        slot = u & (NS - 1)
        wslot = w & 1

        @pl.when(hg == 0)
        def _():
            pltpu.make_async_copy(xbuf.at[blk, b], xbuf.at[blk, b],
                                  x_sems.at[blk * B + b]).wait()

        @pl.when(b == 0)
        def _():
            pltpu.make_async_copy(wqbuf.at[wslot], wqbuf.at[wslot],
                                  w_sems.at[2 * wslot]).wait()
            pltpu.make_async_copy(wobuf.at[wslot], wobuf.at[wslot],
                                  w_sems.at[2 * wslot + 1]).wait()

        pltpu.make_async_copy(kbuf.at[slot], kbuf.at[slot], kv_sems.at[2 * slot]).wait()
        pltpu.make_async_copy(vbuf.at[slot], vbuf.at[slot],
                              kv_sems.at[2 * slot + 1]).wait()

    def compute(u):
        blk, hg, b = dec(u)
        w = u >> lb
        slot = u & (NS - 1)
        wslot = w & 1

        x = xbuf[blk, b]
        q_all = jnp.dot(x, wqbuf[wslot], preferred_element_type=jnp.float32)
        q_all = (q_all * qscale).astype(jnp.bfloat16)

        def qk(g):
            return lax.dot_general(q_all[:, g * Dh:(g + 1) * Dh], kbuf[slot, g],
                                   (((1,), (1,)), ((), ())),
                                   preferred_element_type=jnp.float32)

        def sm_pv(g, s):
            m = jnp.max(s, axis=-1, keepdims=True)
            p = jnp.exp2(s - m)
            l = jnp.sum(p, axis=-1, keepdims=True)
            o = jnp.dot(p.astype(jnp.bfloat16), vbuf[slot, g],
                        preferred_element_type=jnp.float32)
            r = pl.reciprocal(l, approx=True)
            r = r * (2.0 - l * r)
            return (o * r).astype(jnp.bfloat16)

        os_ = []
        s_cur = qk(0)
        for g in range(G):
            s_next = qk(g + 1) if g + 1 < G else None
            os_.append(sm_pv(g, s_cur))
            s_cur = s_next
        o_all = jnp.concatenate(os_, axis=-1)

        prev = jnp.where(hg == 0, 0.0, acc[b])
        new = prev + jnp.dot(o_all, wobuf[wslot], preferred_element_type=jnp.float32)
        acc[b] = new
        obuf[blk, b] = new.astype(obuf.dtype)

    def starts(u, kv=True):
        blk, hg, b = dec(u)
        w = u >> lb

        if kv:
            @pl.when(u + NS < NU)
            def _():
                issue_kv(u + NS)

        @pl.when(jnp.logical_and(b == B - 1, w + 2 < NW))
        def _():
            issue_w(w + 2)

        @pl.when(jnp.logical_and(hg == n_hg - 1, blk == 0))
        def _():
            out_copy(0, b).start()

        @pl.when(jnp.logical_and(hg == n_hg - 1, blk == 1))
        def _():
            out_copy(1, b).start()

    x_copy(xa, 0, 0).start()
    wq_copy(wqa, 0, 0).start()
    start_kv(ka, va, 0, 0, 0)
    wo_copy(woa, 0, 0).start()

    u = jnp.int32(0)
    waits(u)
    static_unit(1)
    wq_copy(wqa, 1, 1).start(priority=1)
    wo_copy(woa, 1, 1).start(priority=1)
    compute(u)
    starts(u, kv=False)
    static_unit(2)
    static_unit(3)

    u = jnp.int32(1)
    waits(u)
    compute(u)
    starts(u, kv=False)

    us = [jnp.int32(2), jnp.int32(3)]
    for u in us:
        waits(u)
    static_unit(4)
    static_unit(5)
    for u in us:
        compute(u)
    for u in us:
        starts(u)
    x_copy(xa, 0, 6).start()
    x_copy(xa, 0, 7).start()
    for b0 in range(B):
        x_copy(xb, 1, b0).start(priority=1)

    def loop_body(i, carry):
        us = [4 + 2 * i, 5 + 2 * i]
        for u in us:
            waits(u)
        for u in us:
            compute(u)
        for u in us:
            starts(u)
        return carry

    lax.fori_loop(0, (NU - 4) // 2, loop_body, 0)

    for blk_s in range(2):
        for b_s in range(B):
            out_copy(blk_s, b_s).wait()


@jax.jit
def pallas_concat_heads__mha_block_cached__mha_block_cached__near_ridge_kernel(
    A_x: jax.Array,
    A_k_cache: jax.Array,
    A_v_cache: jax.Array,
    A_wq: jax.Array,
    A_wo: jax.Array,
    B_x: jax.Array,
    B_k_cache: jax.Array,
    B_v_cache: jax.Array,
    B_wq: jax.Array,
    B_wo: jax.Array,
):
    B, Sq, D = A_x.shape
    _, H, Sk, Dh = A_k_cache.shape
    G, NS = _G, _NS
    kernel = functools.partial(_kernel, B=B, Sq=Sq, D=D, H=H, Sk=Sk, Dh=Dh, G=G, NS=NS)
    any_spec = pl.BlockSpec(memory_space=pl.ANY)
    return pl.pallas_call(
        kernel,
        in_specs=[any_spec] * 10,
        out_specs=any_spec,
        out_shape=jax.ShapeDtypeStruct((B, Sq, 2 * D), A_x.dtype),
        scratch_shapes=[
            pltpu.VMEM((2, B, Sq, D), jnp.bfloat16),
            pltpu.VMEM((NS, G, Sk, Dh), jnp.bfloat16),
            pltpu.VMEM((NS, G, Sk, Dh), jnp.bfloat16),
            pltpu.VMEM((2, D, G * Dh), jnp.bfloat16),
            pltpu.VMEM((2, G * Dh, D), jnp.bfloat16),
            pltpu.VMEM((B, Sq, D), jnp.float32),
            pltpu.VMEM((2, B, Sq, D), jnp.bfloat16),
            pltpu.SemaphoreType.DMA((2 * B,)),
            pltpu.SemaphoreType.DMA((2 * NS,)),
            pltpu.SemaphoreType.DMA((4,)),
            pltpu.SemaphoreType.DMA((2 * B,)),
        ],
        compiler_params=pltpu.CompilerParams(
            vmem_limit_bytes=100 * 1024 * 1024,
        ),
    )(A_x, A_k_cache, A_v_cache, A_wq, A_wo,
      B_x, B_k_cache, B_v_cache, B_wq, B_wo)
```
